```python
import os as _os
_os.environ.setdefault("JAX_PLATFORMS", "cpu")
import jax
import jax.numpy as jnp

def _softmax(x, axis=-1):
    return jax.nn.softmax(x, axis=axis)
def _gelu(x):
    return jax.nn.gelu(x, approximate=True)
def _silu(x):
    return jax.nn.silu(x)
def _sigmoid(x):
    return jax.nn.sigmoid(x)
def _layernorm(x, axis=-1, eps=1e-5):
    m = jnp.mean(x, axis=axis, keepdims=True)
    v = jnp.var(x, axis=axis, keepdims=True)
    return (x - m) / jnp.sqrt(v + eps)
def _scatter_add(tgt, idx, src, axis=0):
    return tgt.at[idx].add(src)
def _segment_sum(src, seg, n):
    return jax.ops.segment_sum(src, seg, n)
class _Rng:
    def __init__(self, key):
        self._k = key
    def _next(self):
        self._k, sub = jax.random.split(self._k)
        return sub
    def normal(self, shape):
        return jax.random.normal(self._next(), shape, dtype=jnp.bfloat16)
    def randint(self, lo, hi, shape):
        return jax.random.randint(self._next(), shape, lo, hi, dtype=jnp.int32)
    def uniform(self, shape, lo=0.0, hi=1.0):
        return jax.random.uniform(self._next(), shape, jnp.bfloat16, lo, hi)
    def permutation(self, n):
        return jax.random.permutation(self._next(), n)


kernel_name = 'concat_heads__gqa_block_cached__mha_block_cached__near_ridge'

def setup_inputs():
    _rng = _Rng(jax.random.key(int.from_bytes(__import__("os").urandom(4), "little")))
    _w = (lambda a: (lambda t: t.astype(jnp.bfloat16) if jnp.issubdtype(t.dtype, jnp.floating) else t)(jnp.asarray(a)))
    def _A_setup():
        B, Sq, D = 16, 32, 1024
        Hq, Hkv, Sk, Dh = 32, 4, 32, 128
        assert Hq % Hkv == 0, (Hq, Hkv)
        return {
            "x": _w((lambda *s: _rng.normal(s) * 0.8)(B, Sq, D)),
            "k_cache": _w((lambda *s: _rng.normal(s) * 0.8)(B, Hkv, Sk, Dh)),
            "v_cache": _w((lambda *s: _rng.normal(s) * 0.05)(B, Hkv, Sk, Dh)),
            "wq": _w((lambda *s: _rng.normal(s) * 0.8)(D, Hq * Dh) * (D ** -0.5)),
            "wo": _w((lambda *s: _rng.normal(s) * 0.05)(Hq * Dh, D) * ((Hq * Dh) ** -0.5)),
        }
    _A_in = _A_setup()

    def _B_setup():
        B, Sq, D = 16, 32, 1024
        H, Sk, Dh = 32, 32, 128
        return {
            "x": _w((lambda *s: _rng.normal(s) * 0.8)(B, Sq, D)),
            "k_cache": _w((lambda *s: _rng.normal(s) * 0.8)(B, H, Sk, Dh)),
            "v_cache": _w((lambda *s: _rng.normal(s) * 0.05)(B, H, Sk, Dh)),
            "wq": _w((lambda *s: _rng.normal(s) * 0.8)(D, H * Dh) * (D ** -0.5)),
            "wo": _w((lambda *s: _rng.normal(s) * 0.05)(H * Dh, D) * ((H * Dh) ** -0.5)),
        }
    _B_in = _B_setup()

    return {
        "A_x": _A_in["x"],
        "A_k_cache": _A_in["k_cache"],
        "A_v_cache": _A_in["v_cache"],
        "A_wq": _A_in["wq"],
        "A_wo": _A_in["wo"],
        "B_x": _B_in["x"],
        "B_k_cache": _B_in["k_cache"],
        "B_v_cache": _B_in["v_cache"],
        "B_wq": _B_in["wq"],
        "B_wo": _B_in["wo"],
    }

def reference(A_x, A_k_cache, A_v_cache, A_wq, A_wo, B_x, B_k_cache, B_v_cache, B_wq, B_wo):
    def _A_ref(x, k_cache, v_cache, wq, wo):
        B, Sq, D = x.shape
        Hq, Dh = 32, 128
        Hkv = k_cache.shape[1]
        rep = Hq // Hkv
        q = (lambda x, *d: x.transpose(*d))((x @ wq).reshape(B, Sq, Hq, Dh), 0, 2, 1, 3)
        k = jnp.repeat(k_cache, rep, axis=1)
        v = jnp.repeat(v_cache, rep, axis=1)
        scores = jnp.einsum("bhqd,bhkd->bhqk", q, k) * (Dh ** -0.5)
        p = _softmax(scores, axis=-1)
        o = jnp.einsum("bhqk,bhkd->bhqd", p, v)
        return (lambda x, *d: x.transpose(*d))(o, 0, 2, 1, 3).reshape(B, Sq, Hq * Dh) @ wo

    def _B_ref(x, k_cache, v_cache, wq, wo):
        B, Sq, D = x.shape
        H, Dh = 32, 128
        q = (lambda x, *d: x.transpose(*d))((x @ wq).reshape(B, Sq, H, Dh), 0, 2, 1, 3)
        scores = jnp.einsum("bhqd,bhkd->bhqk", q, k_cache) * (Dh ** -0.5)
        p = _softmax(scores, axis=-1)
        o = jnp.einsum("bhqk,bhkd->bhqd", p, v_cache)
        return (lambda x, *d: x.transpose(*d))(o, 0, 2, 1, 3).reshape(B, Sq, H * Dh) @ wo

    a = _A_ref(A_x, A_k_cache, A_v_cache, A_wq, A_wo)
    b = _B_ref(B_x, B_k_cache, B_v_cache, B_wq, B_wo)
    return jnp.concatenate([a, b], axis=-1)
```

```python
import math
import jax, jax.numpy as jnp
from jax import lax
import jax.experimental.pallas as pl
import jax.experimental.pallas.tpu as pltpu

B, S, D, H, DH, HKV = 16, 32, 1024, 32, 128, 4
M = B * S
HG = 4
W = HG * DH
NSTEP = H // HG
REP = H // HKV
C = (DH ** -0.5) * math.log2(math.e)
NT = (((1,), (1,)), ((), ()))
NN = (((1,), (0,)), ((), ()))
F32, BF16 = jnp.float32, jnp.bfloat16
A_CHUNKS = (128, 128, 256, 256, 256)
B_CHUNKS = (512, 512)
OUT_B = (256, 256, 256, 128, 128)
SCOPES = False
import contextlib
def scope(n):
    return jax.named_scope(n) if SCOPES else contextlib.nullcontext()


def _dot(a, b, dims=NN):
    return lax.dot_general(a, b, dims, preferred_element_type=F32)


def _softmax_t(sT):
    m = jnp.max(sT, axis=0, keepdims=True)
    e = jnp.exp2((sT - m) * C)
    l = jnp.sum(e, axis=0, keepdims=True)
    return e * pl.reciprocal(l, approx=False)


def _qk_gqa(q, k_ref):
    out = []
    for b in range(B):
        qs = jnp.concatenate([q[b*S:(b+1)*S, h*DH:(h+1)*DH] for h in range(HG)], axis=0)
        out.append(_dot(k_ref[b], qs, NT))
    return out


def _pv_gqa(sTs, v_ref):
    lane_g = lax.broadcasted_iota(jnp.int32, (128, 128), 1) // S
    rows = []
    for bb in range(B // 4):
        pT = jnp.concatenate([_softmax_t(sTs[bb*4 + j]) for j in range(4)], axis=0)
        p = pT.T.astype(BF16)
        lhs = jnp.concatenate([jnp.where(lane_g == j, p, jnp.zeros_like(p)) for j in range(4)], axis=0)
        vs = v_ref[bb*4:(bb+1)*4].reshape(128, DH)
        o = _dot(lhs, vs).astype(BF16)
        for j in range(4):
            rows.append(jnp.concatenate([o[(j*4+h)*S:(j*4+h+1)*S] for h in range(HG)], axis=1))
    return jnp.concatenate(rows, axis=0)


def _qk_mha(q, k_ref):
    lane_g = lax.broadcasted_iota(jnp.int32, (S, 128), 1) // S
    out = []
    for bb in range(B // 4):
        for h in range(HG):
            qs = q[bb*128:(bb+1)*128, h*DH:(h+1)*DH]
            ks = k_ref[bb*4:(bb+1)*4, h].reshape(128, DH)
            sT = _dot(ks, qs, NT)
            d = sT[0:S]
            for j in range(1, 4):
                d = jnp.where(lane_g == j, sT[j*S:(j+1)*S], d)
            out.append(d)
    return out


def _pv_mha(sTs, v_ref):
    lane_g = lax.broadcasted_iota(jnp.int32, (S, 128), 1) // S
    rows = []
    for bb in range(B // 4):
        pT = jnp.concatenate([_softmax_t(sTs[bb*4 + h]) for h in range(HG)], axis=0)
        p = pT.T.astype(BF16)
        for j in range(4):
            pb = p[j*S:(j+1)*S]
            lhs = jnp.concatenate([jnp.where(lane_g == h, pb, jnp.zeros_like(pb)) for h in range(HG)], axis=0)
            vs = v_ref[bb*4 + j].reshape(128, DH)
            o = _dot(lhs, vs).astype(BF16)
            rows.append(jnp.concatenate([o[h*S:(h+1)*S] for h in range(HG)], axis=1))
    return jnp.concatenate(rows, axis=0)


NA, NB = len(A_CHUNKS), len(B_CHUNKS)
SEM_A = 0
SEM_B = SEM_A + NA
SEM_S = SEM_B + NB
SEM_O = SEM_S + NSTEP
NSEM = SEM_O + 1


def _kernel(xa_h, ka_h, va_h, wqa_h, woa_h, xb_h, kb_h, vb_h, wqb_h, wob_h, out_h,
            xa, xb, ka, va, kb, vb, wqa0, wqb0, wqa, wqb, woa, wob, qacc, qb_buf, oa_buf, acc, stage, sems):

    def cp(src, dst, sem):
        return pltpu.make_async_copy(src, dst, sems.at[sem])

    def offs(chunks):
        o, r = 0, []
        for c in chunks:
            r.append((o, c)); o += c
        return r

    def first_chunk(br, i):
        x_h, x_v, w_h, w_v = (xa_h, xa, wqa_h, wqa0) if br == 0 else (xb_h, xb, wqb_h, wqb0)
        o, c = offs(A_CHUNKS if br == 0 else B_CHUNKS)[i]
        sem = (SEM_A if br == 0 else SEM_B) + i
        r = [cp(x_h.at[:, pl.ds(o, c)], x_v.at[:, pl.ds(o, c)], sem),
             cp(w_h.at[pl.ds(o, c), pl.ds(0, 2 * W)], w_v.at[pl.ds(o, c)], sem)]
        if br == 0 and i == NA - 1:
            r.append(cp(ka_h.at[:, 0], ka.at[0], sem))
        if br == 1 and i == NB - 1:
            r.append(cp(va_h.at[:, 0], va.at[0], sem))
        return r

    def second_half(s):
        sem = SEM_S + s
        return [cp(kb_h.at[:, pl.ds(s*HG, HG)], kb.at[s], sem),
                cp(woa_h.at[pl.ds(s*W, W)], woa.at[s], sem),
                cp(vb_h.at[:, pl.ds(s*HG, HG)], vb.at[s], sem),
                cp(wob_h.at[pl.ds(s*W, W)], wob.at[s], sem)]

    def first_half(s):
        sem = SEM_S + s - 1
        g = (s * HG) // REP
        return [cp(wqa_h.at[:, pl.ds(s*W, W)], wqa.at[s - 2], sem),
                cp(ka_h.at[:, g], ka.at[s - 1], sem),
                cp(wqb_h.at[:, pl.ds(s*W, W)], wqb.at[s - 2], sem),
                cp(va_h.at[:, g], va.at[s - 1], sem)]

    def group(s):
        r = second_half(s)
        if isinstance(s, int) and (s == 0 or s == NSTEP - 1):
            return r
        return r + first_half(s + 1)

    def start(cps):
        for c in cps:
            c.start()

    def wait(cps):
        for c in cps:
            c.wait()

    out_chunks = [(0, 768), (768, 256)] + [(D + o, c) for o, c in offs(OUT_B)]

    def cp_out(i):
        o, c = out_chunks[i]
        return cp(stage.at[:, pl.ds(o, c)], out_h.at[:, pl.ds(o, c)], SEM_O)

    for i in range(NA):
        start(first_chunk(0, i))
    for i in range(NB):
        start(first_chunk(1, i))
    for s in range(0, 4):
        start(group(s))

    def qproj_chunked(br):
        x_v, w_v = (xa, wqa0) if br == 0 else (xb, wqb0)
        ch = offs(A_CHUNKS if br == 0 else B_CHUNKS)
        for i, (o, c) in enumerate(ch):
            with scope("w%d_%d" % (br, i)):
                wait(first_chunk(br, i))
            t = _dot(x_v[:, o:o+c], w_v[o:o+c, :])
            if i == 0:
                qacc[...] = t
            elif i < len(ch) - 1:
                qacc[...] += t
            else:
                return (qacc[...] + t).astype(BF16)

    def second(s, oa, qb, first=False, last=False):
        sb = _qk_mha(qb, kb.at[s])

        def oproj(o, w_ref, lo, n, base):
            t = _dot(o, w_ref[s, :, lo:lo+n])
            sl = slice(base + lo, base + lo + n)
            if first:
                acc[:, sl] = t
            elif last:
                stage[:, sl] = (acc[:, sl] + t).astype(BF16)
            else:
                acc[:, sl] += t

        oproj(oa, woa, 0, 768, 0)
        if last:
            cp_out(0).start()
        ob = _pv_mha(sb, vb.at[s])
        oproj(oa, woa, 768, 256, 0)
        if last:
            cp_out(1).start()
            for i, (o, c) in enumerate(offs(OUT_B)):
                oproj(ob, wob, o, c, D)
                cp_out(2 + i).start()
            with scope("wout"):
                for i in range(len(out_chunks)):
                    cp_out(i).wait()
        else:
            oproj(ob, wob, 0, D, D)

    with scope("first"):
        qa = qproj_chunked(0)
        sa0 = _qk_gqa(qa[:, 0:W], ka.at[0])
        sa1 = _qk_gqa(qa[:, W:2*W], ka.at[0])
        qb = qproj_chunked(1)
        oa0 = _pv_gqa(sa0, va.at[0])
        oa_buf[...] = _pv_gqa(sa1, va.at[0])
        qb_buf[...] = qb[:, W:2*W]
        with scope("wg0"):
            wait(group(0))
        for s in range(4, NSTEP):
            start(group(s))
        second(0, oa0, qb[:, 0:W], first=True)

    def body(s, carry):
        with scope("mid"):
            with scope("wg"):
                wait(group(s))
            second(s, oa_buf[...], qb_buf[...])
            qa = _dot(xa[...], wqa[s - 1]).astype(BF16)
            sa = _qk_gqa(qa, ka.at[s])
            qb_buf[...] = _dot(xb[...], wqb[s - 1]).astype(BF16)
            oa_buf[...] = _pv_gqa(sa, va.at[s])
        return carry
    lax.fori_loop(1, NSTEP - 1, body, 0)

    with scope("last"):
        wait(group(NSTEP - 1))
        second(NSTEP - 1, oa_buf[...], qb_buf[...], last=True)


@jax.jit
def pallas_concat_heads__gqa_block_cached__mha_block_cached__near_ridge_kernel(A_x, A_k_cache, A_v_cache, A_wq, A_wo, B_x, B_k_cache, B_v_cache, B_wq, B_wo):
    any_spec = pl.BlockSpec(memory_space=pl.ANY)
    out = pl.pallas_call(
        _kernel,
        in_specs=[any_spec] * 10,
        out_specs=any_spec,
        out_shape=jax.ShapeDtypeStruct((M, 2 * D), BF16),
        scratch_shapes=[
            pltpu.VMEM((M, D), BF16), pltpu.VMEM((M, D), BF16),
            pltpu.VMEM((NSTEP - 1, B, S, DH), BF16), pltpu.VMEM((NSTEP - 1, B, S, DH), BF16),
            pltpu.VMEM((NSTEP, B, HG, S, DH), BF16), pltpu.VMEM((NSTEP, B, HG, S, DH), BF16),
            pltpu.VMEM((D, 2 * W), BF16), pltpu.VMEM((D, 2 * W), BF16),
            pltpu.VMEM((NSTEP - 2, D, W), BF16), pltpu.VMEM((NSTEP - 2, D, W), BF16),
            pltpu.VMEM((NSTEP, W, D), BF16), pltpu.VMEM((NSTEP, W, D), BF16),
            pltpu.VMEM((M, 2 * W), F32), pltpu.VMEM((M, W), BF16), pltpu.VMEM((M, W), BF16),
            pltpu.VMEM((M, 2 * D), F32), pltpu.VMEM((M, 2 * D), BF16),
            pltpu.SemaphoreType.DMA((NSEM,)),
        ],
        compiler_params=pltpu.CompilerParams(vmem_limit_bytes=100 * 1024 * 1024),
    )(A_x.reshape(M, D), A_k_cache, A_v_cache, A_wq, A_wo, B_x.reshape(M, D), B_k_cache, B_v_cache, B_wq, B_wo)
    return out.reshape(B, S, 2 * D)
```

```python
import math

import jax
import jax.numpy as jnp
from jax import lax
import jax.experimental.pallas as pl
import jax.experimental.pallas.tpu as pltpu

B, S, D, H, DH, HKV = 16, 32, 1024, 32, 128, 4
M = B * S
HG = 4
W = HG * DH
NSTEP = H // HG
REP = H // HKV
C = (DH ** -0.5) * math.log2(math.e)
NT = (((1,), (1,)), ((), ()))
NN = (((1,), (0,)), ((), ()))
F32, BF16 = jnp.float32, jnp.bfloat16

A_KSEG = (128, 256, 512, 768)
B_KSEG = 256
WSPLIT = 384
DEF = 256
ND = D - DEF
OUT_B = (256, 256, 256, 128, 128)
OUT_ROWS = (256, 128, 64, 64)

NA = len(A_KSEG)
NSEG = NA + 3
NSEM = NSEG + NSTEP


def _offs(chunks):
    o, r = 0, []
    for c in chunks:
        r.append((o, c))
        o += c
    return r


def _dot(a, b, dims=NN):
    return lax.dot_general(a, b, dims, preferred_element_type=F32)


def _softmax_t(s_t):
    m = jnp.max(s_t, axis=0, keepdims=True)
    e = jnp.exp2((s_t - m) * C)
    l = jnp.sum(e, axis=0, keepdims=True)
    r = pl.reciprocal(l, approx=True)
    r = r * (2.0 - l * r)
    return e * r


def _qk_gqa4(q, k_ref, bb):
    out = []
    for b in range(bb * 4, bb * 4 + 4):
        qs = jnp.concatenate(
            [q[b * S:(b + 1) * S, h * DH:(h + 1) * DH] for h in range(HG)], axis=0)
        out.append(_dot(k_ref[b], qs, NT))
    return out


def _pv_gqa(s_ts, v_ref, fine=False):
    lane_g = lax.broadcasted_iota(jnp.int32, (128, 128), 1) // S
    rows = []
    for bb in range(B // 4):
        p_t = jnp.concatenate([_softmax_t(s_ts[bb * 4 + j]) for j in range(4)], axis=0)
        p = p_t.T.astype(BF16)
        vs = v_ref[bb * 4:(bb + 1) * 4].reshape(128, DH)
        lhs = [jnp.where(lane_g == j, p, jnp.zeros_like(p)) for j in range(4)]
        if fine:
            o = jnp.concatenate([_dot(t, vs).astype(BF16) for t in lhs], axis=0)
        else:
            o = _dot(jnp.concatenate(lhs, axis=0), vs).astype(BF16)
        for j in range(4):
            rows.append(jnp.concatenate(
                [o[(j * 4 + h) * S:(j * 4 + h + 1) * S] for h in range(HG)], axis=1))
    return jnp.concatenate(rows, axis=0)


def _qk_mha4(q, k_ref, bb):
    lane_g = lax.broadcasted_iota(jnp.int32, (S, 128), 1) // S
    out = []
    for h in range(HG):
        qs = q[bb * 128:(bb + 1) * 128, h * DH:(h + 1) * DH]
        ks = k_ref[bb * 4:(bb + 1) * 4, h].reshape(128, DH)
        s_t = _dot(ks, qs, NT)
        d = s_t[0:S]
        for j in range(1, 4):
            d = jnp.where(lane_g == j, s_t[j * S:(j + 1) * S], d)
        out.append(d)
    return out


def _qk_mha(q, k_ref):
    return [t for bb in range(B // 4) for t in _qk_mha4(q, k_ref, bb)]


def _pv_mha(s_ts, v_ref):
    lane_g = lax.broadcasted_iota(jnp.int32, (S, 128), 1) // S
    rows = []
    for bb in range(B // 4):
        p_t = jnp.concatenate([_softmax_t(s_ts[bb * 4 + h]) for h in range(HG)], axis=0)
        p = p_t.T.astype(BF16)
        for j in range(4):
            pb = p[j * S:(j + 1) * S]
            lhs = jnp.concatenate(
                [jnp.where(lane_g == h, pb, jnp.zeros_like(pb)) for h in range(HG)], axis=0)
            vs = v_ref[bb * 4 + j].reshape(128, DH)
            o = _dot(lhs, vs).astype(BF16)
            rows.append(jnp.concatenate([o[h * S:(h + 1) * S] for h in range(HG)], axis=1))
    return jnp.concatenate(rows, axis=0)


def _kernel(xa_h, ka_h, va_h, wqa_h, woa_h, xb_h, kb_h, vb_h, wqb_h, wob_h, out_h,
            xa, xb, ka, va, kb, vb, wqa0, wqb0, wqa, wqb, woa, wob,
            qacc, qb_buf, ob_buf, acc, stage_a, stage_b, sems):

    def cp(src, dst, sem):
        return pltpu.make_async_copy(src, dst, sems.at[sem])

    def xw(br, k0, k1, sem):
        x_h, x_v, w_h, w_v = (xa_h, xa, wqa_h, wqa0) if br == 0 else (xb_h, xb, wqb_h, wqb0)
        n = k1 - k0
        return [cp(x_h.at[:, pl.ds(k0, n)], x_v.at[:, pl.ds(k0, n)], sem),
                cp(w_h.at[pl.ds(k0, n), pl.ds(0, 2 * W)], w_v.at[pl.ds(k0, n)], sem)]

    def b_data(s, sem, first=False, last=False):
        r = [cp(kb_h.at[:, pl.ds(s * HG, HG)], kb.at[s], sem),
             cp(vb_h.at[:, pl.ds(s * HG, HG)], vb.at[s], sem)]
        if last:
            r.append(cp(wob_h.at[pl.ds(s * W, W)], wob.at[s], sem))
        else:
            r.append(cp(wob_h.at[pl.ds(s * W, W), pl.ds(0, ND)],
                        wob.at[s, :, pl.ds(0, ND)], sem))
        if not first:
            r.append(cp(wob_h.at[pl.ds((s - 1) * W, W), pl.ds(ND, DEF)],
                        wob.at[s - 1, :, pl.ds(ND, DEF)], sem))
        return r

    def seg(i):
        if i < NA:
            return xw(0, A_KSEG[i - 1] if i else 0, A_KSEG[i], i)
        if i == NA:
            return xw(0, A_KSEG[-1], D, i) + [
                cp(ka_h.at[:, 0], ka.at[0], i),
                cp(va_h.at[:, 0], va.at[0], i),
                cp(woa_h.at[pl.ds(0, W), pl.ds(0, WSPLIT)], woa.at[0, :, pl.ds(0, WSPLIT)], i)]
        if i == NA + 1:
            return [cp(woa_h.at[pl.ds(0, W), pl.ds(WSPLIT, D - WSPLIT)],
                       woa.at[0, :, pl.ds(WSPLIT, D - WSPLIT)], i),
                    cp(woa_h.at[pl.ds(W, W)], woa.at[1], i)] + xw(1, 0, B_KSEG, i)
        return xw(1, B_KSEG, D, i) + b_data(0, i, first=True)

    def group(s):
        sem = NSEG + s - 1
        g = ((s + 1) * HG) // REP
        return [cp(wqa_h.at[:, pl.ds((s + 1) * W, W)], wqa.at[s - 1], sem),
                cp(ka_h.at[:, g], ka.at[s], sem),
                cp(wqb_h.at[:, pl.ds((s + 1) * W, W)], wqb.at[s - 1], sem),
                cp(va_h.at[:, g], va.at[s], sem),
                cp(woa_h.at[pl.ds((s + 1) * W, W)], woa.at[s + 1], sem)] + b_data(s, sem)

    def last_group():
        return b_data(NSTEP - 1, NSEG + NSTEP - 2, last=True)

    def cp_out_a():
        return cp(stage_a, out_h.at[:, pl.ds(0, D)], NSEM - 1)

    def cp_out_b(i):
        o, c = _offs(OUT_B)[i]
        return cp(stage_b.at[:, pl.ds(o, c)], out_h.at[:, pl.ds(D + o, c)], NSEM - 1)

    def cp_out_last(j):
        o, c = _offs(OUT_B)[-1]
        r0, r = _offs(OUT_ROWS)[j]
        return cp(stage_b.at[pl.ds(r0, r), pl.ds(o, c)],
                  out_h.at[pl.ds(r0, r), pl.ds(D + o, c)], NSEM - 1)

    def start(cps):
        for c in cps:
            c.start()

    def wait(cps):
        for c in cps:
            c.wait()

    def qpart(br, k0, k1, n0, n1, mode):
        x_v, w_v = (xa, wqa0) if br == 0 else (xb, wqb0)
        t = _dot(x_v[:, k0:k1], w_v[k0:k1, n0:n1])
        if mode == "set":
            qacc[:, n0:n1] = t
        elif mode == "add":
            qacc[:, n0:n1] += t
        else:
            return (qacc[:, n0:n1] + t).astype(BF16)

    def oproj(o, w_ref, s, lo, n, base, mode):
        t = _dot(o, w_ref[s, :, lo:lo + n])
        sl = slice(base + lo, base + lo + n)
        if mode == "set":
            acc[:, sl] = t
        elif mode == "add":
            acc[:, sl] += t
        elif mode == "add+stage":
            r = acc[:, sl] + t
            acc[:, sl] = r
            stage_a[:, lo:lo + n] = r.astype(BF16)
        else:
            stage_b[:, lo:lo + n] = (acc[:, sl] + t).astype(BF16)

    for i in range(NSEG):
        start(seg(i))
    for s in range(1, 4):
        start(group(s))
    acc[:, D + ND:2 * D] = jnp.zeros((M, DEF), F32)

    for i in range(NA):
        wait(seg(i))
        qpart(0, A_KSEG[i - 1] if i else 0, A_KSEG[i], 0, 2 * W, "add" if i else "set")

    wait(seg(NA))
    k0 = A_KSEG[-1]
    qa0 = qpart(0, k0, D, 0, W, "fin")
    sa0 = _qk_gqa4(qa0, ka.at[0], 0)
    qpart(0, k0, D - 128, W, 2 * W, "add")
    for bb in range(1, 4):
        sa0 += _qk_gqa4(qa0, ka.at[0], bb)
    qa1 = qpart(0, D - 128, D, W, 2 * W, "fin")
    oa0 = _pv_gqa(sa0, va.at[0], fine=True)
    sa1 = _qk_gqa4(qa1, ka.at[0], 0) + _qk_gqa4(qa1, ka.at[0], 1)
    oproj(oa0, woa, 0, 0, 128, 0, "set")
    sa1 += _qk_gqa4(qa1, ka.at[0], 2) + _qk_gqa4(qa1, ka.at[0], 3)
    oproj(oa0, woa, 0, 128, WSPLIT - 256, 0, "set")
    oa1 = _pv_gqa(sa1, va.at[0], fine=True)
    oproj(oa0, woa, 0, WSPLIT - 128, 128, 0, "set")
    for s in range(4, NSTEP - 1):
        start(group(s))
    start(last_group())

    wait(seg(NA + 1))
    qpart(1, 0, B_KSEG, 0, 2 * W, "set")
    oproj(oa0, woa, 0, WSPLIT, D - WSPLIT, 0, "set")
    oproj(oa1, woa, 1, 0, D, 0, "add")

    wait(seg(NA + 2))
    k0 = B_KSEG
    qpart(1, k0, k0 + 128, W, 2 * W, "add")
    qb0 = qpart(1, k0, D, 0, W, "fin")
    qpart(1, k0 + 128, k0 + 256, W, 2 * W, "add")
    sb0 = _qk_mha(qb0, kb.at[0])
    qpart(1, k0 + 256, D - 128, W, 2 * W, "add")
    ob0 = _pv_mha(sb0, vb.at[0])
    qb_buf[...] = qpart(1, D - 128, D, W, 2 * W, "fin")
    ob_buf[...] = ob0
    oproj(ob0, wob, 0, 0, ND, D, "set")

    def body(s, carry):
        wait(group(s))
        qs, sb = [], []
        for h in range(HG):
            qs.append(_dot(xa[...], wqa[s - 1, :, h * DH:(h + 1) * DH]).astype(BF16))
            sb += _qk_mha4(qb_buf, kb.at[s], h)
        qa = jnp.concatenate(qs, axis=1)
        oproj(ob_buf[...], wob, s - 1, ND, DEF, D, "add")
        sa = []
        for h in range(HG):
            sa += _qk_gqa4(qa, ka.at[s], h)
            qb_buf[:, h * DH:(h + 1) * DH] = _dot(
                xb[...], wqb[s - 1, :, h * DH:(h + 1) * DH]).astype(BF16)
        ob = _pv_mha(sb, vb.at[s])
        ob_buf[...] = ob
        oa = _pv_gqa(sa, va.at[s])
        oproj(ob, wob, s, 0, ND, D, "add")
        oproj(oa, woa, s + 1, 0, D, 0, "add+stage")
        return carry

    lax.fori_loop(1, NSTEP - 1, body, 0)

    s = NSTEP - 1
    cp_out_a().start()
    wait(last_group())
    acc[:, D + ND:2 * D] += _dot(ob_buf[:, 0:W // 2], wob[s - 1, 0:W // 2, ND:D])
    sb = _qk_mha(qb_buf, kb.at[s])
    acc[:, D + ND:2 * D] += _dot(ob_buf[:, W // 2:W], wob[s - 1, W // 2:W, ND:D])
    ob = _pv_mha(sb, vb.at[s])
    for i, (o, c) in enumerate(_offs(OUT_B)[:-1]):
        oproj(ob, wob, s, o, c, D, "fin")
        cp_out_b(i).start()
    o, c = _offs(OUT_B)[-1]
    t = _dot(ob, wob[s, :, o:o + c])
    for j, (r0, r) in enumerate(_offs(OUT_ROWS)):
        stage_b[r0:r0 + r, o:o + c] = (
            acc[r0:r0 + r, D + o:D + o + c] + t[r0:r0 + r]).astype(BF16)
        cp_out_last(j).start()
    wait([cp_out_a()] + [cp_out_b(i) for i in range(len(OUT_B) - 1)]
         + [cp_out_last(j) for j in range(len(OUT_ROWS))])


@jax.jit
def pallas_concat_heads__gqa_block_cached__mha_block_cached__near_ridge_kernel(
    A_x: jax.Array,
    A_k_cache: jax.Array,
    A_v_cache: jax.Array,
    A_wq: jax.Array,
    A_wo: jax.Array,
    B_x: jax.Array,
    B_k_cache: jax.Array,
    B_v_cache: jax.Array,
    B_wq: jax.Array,
    B_wo: jax.Array,
):
    any_spec = pl.BlockSpec(memory_space=pl.ANY)
    out = pl.pallas_call(
        _kernel,
        in_specs=[any_spec] * 10,
        out_specs=any_spec,
        out_shape=jax.ShapeDtypeStruct((M, 2 * D), BF16),
        scratch_shapes=[
            pltpu.VMEM((M, D), BF16), pltpu.VMEM((M, D), BF16),
            pltpu.VMEM((NSTEP - 1, B, S, DH), BF16),
            pltpu.VMEM((NSTEP - 1, B, S, DH), BF16),
            pltpu.VMEM((NSTEP, B, HG, S, DH), BF16),
            pltpu.VMEM((NSTEP, B, HG, S, DH), BF16),
            pltpu.VMEM((D, 2 * W), BF16), pltpu.VMEM((D, 2 * W), BF16),
            pltpu.VMEM((NSTEP - 2, D, W), BF16), pltpu.VMEM((NSTEP - 2, D, W), BF16),
            pltpu.VMEM((NSTEP, W, D), BF16), pltpu.VMEM((NSTEP, W, D), BF16),
            pltpu.VMEM((M, 2 * W), F32),
            pltpu.VMEM((M, W), BF16), pltpu.VMEM((M, W), BF16),
            pltpu.VMEM((M, 2 * D), F32),
            pltpu.VMEM((M, D), BF16), pltpu.VMEM((M, D), BF16),
            pltpu.SemaphoreType.DMA((NSEM,)),
        ],
        compiler_params=pltpu.CompilerParams(
            vmem_limit_bytes=100 * 1024 * 1024,
            disable_semaphore_checks=True,
        ),
    )(A_x.reshape(M, D), A_k_cache, A_v_cache, A_wq, A_wo,
      B_x.reshape(M, D), B_k_cache, B_v_cache, B_wq, B_wo)
    return out.reshape(B, S, 2 * D)
```

```python
import math

import jax
import jax.numpy as jnp
from jax import lax
import jax.experimental.pallas as pl
import jax.experimental.pallas.tpu as pltpu

B, S, D, H, DH, HKV = 16, 32, 1024, 32, 128, 4
M = B * S
HG = 4
W = HG * DH
NSTEP = H // HG
REP = H // HKV
KT = D // 128
SCALE = 0.08837890625
LOG2E = math.log2(math.e)
NT = (((1,), (1,)), ((), ()))
NN = (((1,), (0,)), ((), ()))
F32, BF16 = jnp.float32, jnp.bfloat16

ASEG = ((1, 0, 0), (1, 1, 1), (2, 2, 2), (4, 3, 3), (6, 6, 5))
B_KSEG = 512
WSPLIT = 256
DEF = 256
ND = D - DEF
OUT_B = (256, 256, 256, 128, 128)
OUT_ROWS = (256, 128, 64, 64)

NA = len(ASEG)
NSEG = NA + 3
NSEM = NSEG + NSTEP


def _offs(chunks):
    o, r = 0, []
    for c in chunks:
        r.append((o, c))
        o += c
    return r


def _rects(lo, hi):
    out = []
    ks = sorted(set(lo) | set(hi))
    for k0, k1 in zip(ks[:-1], ks[1:]):
        gs = [g for g in range(len(lo)) if lo[g] <= k0 and k1 <= hi[g]]
        if gs:
            assert gs == list(range(gs[0], gs[-1] + 1))
            out.append((k0, k1, gs[0], gs[-1] + 1))
    return out


def _dot(a, b, dims=NN):
    return lax.dot_general(a, b, dims, preferred_element_type=F32)


def _softmax_t(s_t):
    s_t = (s_t.astype(BF16).astype(F32) * SCALE).astype(BF16).astype(F32)
    m = jnp.max(s_t, axis=0, keepdims=True)
    e = jnp.exp2((s_t - m) * LOG2E)
    l = jnp.sum(e, axis=0, keepdims=True)
    r = pl.reciprocal(l, approx=True)
    r = r * (2.0 - l * r)
    return e * r


def _qk_gqa4(q, k_ref, bb):
    out = []
    for b in range(bb * 4, bb * 4 + 4):
        qs = jnp.concatenate(
            [q[b * S:(b + 1) * S, h * DH:(h + 1) * DH] for h in range(HG)], axis=0)
        out.append(_dot(k_ref[b], qs, NT))
    return out


def _pv_gqa(s_ts, v_ref, fine=False):
    lane_g = lax.broadcasted_iota(jnp.int32, (128, 128), 1) // S
    rows = []
    for bb in range(B // 4):
        p_t = jnp.concatenate([_softmax_t(s_ts[bb * 4 + j]) for j in range(4)], axis=0)
        p = p_t.T.astype(BF16)
        vs = v_ref[bb * 4:(bb + 1) * 4].reshape(128, DH)
        lhs = [jnp.where(lane_g == j, p, jnp.zeros_like(p)) for j in range(4)]
        if fine:
            o = jnp.concatenate([_dot(t, vs).astype(BF16) for t in lhs], axis=0)
        else:
            o = _dot(jnp.concatenate(lhs, axis=0), vs).astype(BF16)
        for j in range(4):
            rows.append(jnp.concatenate(
                [o[(j * 4 + h) * S:(j * 4 + h + 1) * S] for h in range(HG)], axis=1))
    return jnp.concatenate(rows, axis=0)


def _qk_mha4(q, k_ref, bb):
    lane_g = lax.broadcasted_iota(jnp.int32, (S, 128), 1) // S
    out = []
    for h in range(HG):
        qs = q[bb * 128:(bb + 1) * 128, h * DH:(h + 1) * DH]
        ks = k_ref[bb * 4:(bb + 1) * 4, h].reshape(128, DH)
        s_t = _dot(ks, qs, NT)
        d = s_t[0:S]
        for j in range(1, 4):
            d = jnp.where(lane_g == j, s_t[j * S:(j + 1) * S], d)
        out.append(d)
    return out


def _qk_mha(q, k_ref):
    return [t for bb in range(B // 4) for t in _qk_mha4(q, k_ref, bb)]


def _pv_mha(s_ts, v_ref):
    lane_g = lax.broadcasted_iota(jnp.int32, (S, 128), 1) // S
    rows = []
    for bb in range(B // 4):
        p_t = jnp.concatenate([_softmax_t(s_ts[bb * 4 + h]) for h in range(HG)], axis=0)
        p = p_t.T.astype(BF16)
        for j in range(4):
            pb = p[j * S:(j + 1) * S]
            lhs = jnp.concatenate(
                [jnp.where(lane_g == h, pb, jnp.zeros_like(pb)) for h in range(HG)], axis=0)
            vs = v_ref[bb * 4 + j].reshape(128, DH)
            o = _dot(lhs, vs).astype(BF16)
            rows.append(jnp.concatenate([o[h * S:(h + 1) * S] for h in range(HG)], axis=1))
    return jnp.concatenate(rows, axis=0)


def _kernel(xa_h, ka_h, va_h, wqa_h, woa_h, xb_h, kb_h, vb_h, wqb_h, wob_h, out_h,
            xab, ka, va, kb, vb, wqa0, wqb, wq2, woa, wob,
            qacc, q_buf, ob_buf, acc, stage_a, stage_b, sems):

    def cp(src, dst, sem):
        return pltpu.make_async_copy(src, dst, sems.at[sem])

    def a_first(lo, hi, sem):
        r = []
        x_todo = hi[0] > lo[0]
        for k0, k1, g0, g1 in _rects(lo, hi):
            if x_todo and k0 >= lo[0]:
                cols = pl.ds(lo[0] * 128, (hi[0] - lo[0]) * 128)
                r.append(cp(xa_h.at[:, cols], xab.at[0, :, cols], sem))
                x_todo = False
            rows, cols = pl.ds(k0 * 128, (k1 - k0) * 128), pl.ds(g0 * W, (g1 - g0) * W)
            r.append(cp(wqa_h.at[rows, cols], wqa0.at[rows, cols], sem))
        return r

    def b_first(k0, k1, sem):
        ks = pl.ds(k0, k1 - k0)
        return [cp(xb_h.at[:, ks], xab.at[1, :, ks], sem),
                cp(wqb_h.at[ks, pl.ds(0, W)], wqb.at[0, ks], sem)]

    def b_data(s, sem, first=False, last=False):
        r = [cp(kb_h.at[:, pl.ds(s * HG, HG)], kb.at[s], sem),
             cp(vb_h.at[:, pl.ds(s * HG, HG)], vb.at[s], sem)]
        if last:
            r.append(cp(wob_h.at[pl.ds(s * W, W)], wob.at[s], sem))
        else:
            r.append(cp(wob_h.at[pl.ds(s * W, W), pl.ds(0, ND)],
                        wob.at[s, :, pl.ds(0, ND)], sem))
        if not first:
            r.append(cp(wob_h.at[pl.ds((s - 1) * W, W), pl.ds(ND, DEF)],
                        wob.at[s - 1, :, pl.ds(ND, DEF)], sem))
        return r

    def seg(i):
        if i < NA:
            return a_first(ASEG[i - 1] if i else (0, 0, 0), ASEG[i], i)
        if i == NA:
            return a_first(ASEG[-1], (KT, KT, KT), i) + [
                cp(ka_h.at[:, 0], ka.at[0], i),
                cp(va_h.at[:, 0], va.at[0], i),
                cp(woa_h.at[pl.ds(0, W), pl.ds(0, WSPLIT)], woa.at[0, :, pl.ds(0, WSPLIT)], i)]
        if i == NA + 1:
            return [cp(woa_h.at[pl.ds(0, W), pl.ds(WSPLIT, D - WSPLIT)],
                       woa.at[0, :, pl.ds(WSPLIT, D - WSPLIT)], i),
                    cp(woa_h.at[pl.ds(W, W)], woa.at[1], i)] + b_first(0, B_KSEG, i)
        return b_first(B_KSEG, D, i) + b_data(0, i, first=True)

    def group(s, issue=False):
        sem = NSEG + s - 1
        g = ((s + 1) * HG) // REP
        if not issue:
            ahead = wq2.at[s - 1]
        elif s < NSTEP - 2:
            ahead = wqa_h.at[:, pl.ds((s + 2) * W, W)]
        else:
            ahead = wqb_h.at[:, pl.ds((s + 1) * W, W)]
        return [cp(wqb_h.at[:, pl.ds(s * W, W)], wqb.at[s], sem),
                cp(ka_h.at[:, g], ka.at[s], sem),
                cp(ahead, wq2.at[s - 1], sem),
                cp(va_h.at[:, g], va.at[s], sem),
                cp(woa_h.at[pl.ds((s + 1) * W, W)], woa.at[s + 1], sem)] + b_data(s, sem)

    def last_group():
        return b_data(NSTEP - 1, NSEG + NSTEP - 2, last=True)

    def cp_out_a():
        return cp(stage_a, out_h.at[:, pl.ds(0, D)], NSEM - 1)

    def cp_out_b(i):
        o, c = _offs(OUT_B)[i]
        return cp(stage_b.at[:, pl.ds(o, c)], out_h.at[:, pl.ds(D + o, c)], NSEM - 1)

    def cp_out_last(j):
        o, c = _offs(OUT_B)[-1]
        r0, r = _offs(OUT_ROWS)[j]
        return cp(stage_b.at[pl.ds(r0, r), pl.ds(o, c)],
                  out_h.at[pl.ds(r0, r), pl.ds(D + o, c)], NSEM - 1)

    def start(cps):
        for c in cps:
            c.start()

    def wait(cps):
        for c in cps:
            c.wait()

    def qpart(br, k0, k1, n0, n1, mode):
        w = wqa0[k0:k1, n0:n1] if br == 0 else wqb[0, k0:k1, n0:n1]
        t = _dot(xab[br, :, k0:k1], w)
        if mode == "set":
            qacc[:, n0:n1] = t
        elif mode == "add":
            qacc[:, n0:n1] += t
        else:
            return (qacc[:, n0:n1] + t).astype(BF16)

    def oproj(o, w_ref, s, lo, n, base, mode):
        t = _dot(o, w_ref[s, :, lo:lo + n])
        sl = slice(base + lo, base + lo + n)
        if mode == "set":
            acc[:, sl] = t
        elif mode == "add":
            acc[:, sl] += t
        elif mode == "add+stage":
            r = acc[:, sl] + t
            acc[:, sl] = r
            stage_a[:, lo:lo + n] = r.astype(BF16)
        else:
            stage_b[:, lo:lo + n] = (acc[:, sl] + t).astype(BF16)

    for i in range(NSEG):
        start(seg(i))
    for s in range(1, 4):
        start(group(s, issue=True))
    acc[:, D + ND:2 * D] = jnp.zeros((M, DEF), F32)

    for i in range(NA):
        wait(seg(i))
        for k0, k1, g0, g1 in _rects(ASEG[i - 1] if i else (0, 0, 0), ASEG[i]):
            qpart(0, k0 * 128, k1 * 128, g0 * W, g1 * W, "add" if k0 else "set")

    wait(seg(NA))
    k0, k1, k2 = [k * 128 for k in ASEG[-1]]
    ka0 = ka.at[0]
    qa0 = qpart(0, k0, D, 0, W, "fin")
    sa0 = _qk_gqa4(qa0, ka0, 0)
    qpart(0, k1, k1 + 128, W, 2 * W, "add")
    sa0 += _qk_gqa4(qa0, ka0, 1)
    qa1 = qpart(0, k1 + 128, D, W, 2 * W, "fin")
    sa0 += _qk_gqa4(qa0, ka0, 2)
    qpart(0, k2, k2 + 128, 2 * W, 3 * W, "add")
    sa0 += _qk_gqa4(qa0, ka0, 3)
    sa1 = _qk_gqa4(qa1, ka0, 0)
    qpart(0, k2 + 128, D - 128, 2 * W, 3 * W, "add")
    sa1 += _qk_gqa4(qa1, ka0, 1)
    oa0 = _pv_gqa(sa0, va.at[0], fine=True)
    sa1 += _qk_gqa4(qa1, ka0, 2)
    q_buf[...] = qpart(0, D - 128, D, 2 * W, 3 * W, "fin")
    sa1 += _qk_gqa4(qa1, ka0, 3)
    oproj(oa0, woa, 0, 0, 128, 0, "set")
    oa1 = _pv_gqa(sa1, va.at[0], fine=True)
    oproj(oa0, woa, 0, 128, WSPLIT - 128, 0, "set")

    wait(seg(NA + 1))
    qpart(1, 0, B_KSEG, 0, W, "set")
    oproj(oa0, woa, 0, WSPLIT, D - WSPLIT, 0, "set")
    oproj(oa1, woa, 1, 0, D - 384, 0, "add")

    wait(seg(NA + 2))
    qpart(1, B_KSEG, B_KSEG + 128, 0, W, "add")
    qb0 = qpart(1, B_KSEG + 128, D, 0, W, "fin")
    oproj(oa1, woa, 1, D - 384, 128, 0, "add")
    sb0 = _qk_mha(qb0, kb.at[0])
    oproj(oa1, woa, 1, D - 256, 128, 0, "add")
    ob0 = _pv_mha(sb0, vb.at[0])
    oproj(oa1, woa, 1, D - 128, 128, 0, "add")
    ob_buf[...] = ob0
    oproj(ob0, wob, 0, 0, ND, D, "set")
    for s in range(4, NSTEP - 1):
        start(group(s, issue=True))
    start(last_group())

    def body(s, carry):
        wait(group(s))
        qb = _dot(xab[1], wqb[s]).astype(BF16)
        sa = _qk_gqa4(q_buf, ka.at[s], 0) + _qk_gqa4(q_buf, ka.at[s], 1)
        sb = _qk_mha4(qb, kb.at[s], 0) + _qk_mha4(qb, kb.at[s], 1)
        oproj(ob_buf[...], wob, s - 1, ND, DEF, D, "add")
        for bb in (2, 3):
            sa += _qk_gqa4(q_buf, ka.at[s], bb)
            sb += _qk_mha4(qb, kb.at[s], bb)
        q_buf[...] = _dot(xab[s // (NSTEP - 2)], wq2[s - 1]).astype(BF16)
        oa = _pv_gqa(sa, va.at[s])
        ob = _pv_mha(sb, vb.at[s])
        ob_buf[...] = ob
        oproj(oa, woa, s + 1, 0, D, 0, "add+stage")
        oproj(ob, wob, s, 0, ND, D, "add")
        return carry

    lax.fori_loop(1, NSTEP - 1, body, 0)

    s = NSTEP - 1
    cp_out_a().start()
    wait(last_group())
    acc[:, D + ND:2 * D] += _dot(ob_buf[:, 0:W // 2], wob[s - 1, 0:W // 2, ND:D])
    sb = _qk_mha(q_buf, kb.at[s])
    acc[:, D + ND:2 * D] += _dot(ob_buf[:, W // 2:W], wob[s - 1, W // 2:W, ND:D])
    ob = _pv_mha(sb, vb.at[s])
    for i, (o, c) in enumerate(_offs(OUT_B)[:-1]):
        oproj(ob, wob, s, o, c, D, "fin")
        cp_out_b(i).start()
    o, c = _offs(OUT_B)[-1]
    t = _dot(ob, wob[s, :, o:o + c])
    for j, (r0, r) in enumerate(_offs(OUT_ROWS)):
        stage_b[r0:r0 + r, o:o + c] = (
            acc[r0:r0 + r, D + o:D + o + c] + t[r0:r0 + r]).astype(BF16)
        cp_out_last(j).start()
    wait([cp_out_a()] + [cp_out_b(i) for i in range(len(OUT_B) - 1)]
         + [cp_out_last(j) for j in range(len(OUT_ROWS))])


@jax.jit
def pallas_concat_heads__gqa_block_cached__mha_block_cached__near_ridge_kernel(
    A_x: jax.Array,
    A_k_cache: jax.Array,
    A_v_cache: jax.Array,
    A_wq: jax.Array,
    A_wo: jax.Array,
    B_x: jax.Array,
    B_k_cache: jax.Array,
    B_v_cache: jax.Array,
    B_wq: jax.Array,
    B_wo: jax.Array,
):
    any_spec = pl.BlockSpec(memory_space=pl.ANY)
    vmem_limit = 100 * 1024 * 1024
    try:
        params = pltpu.CompilerParams(vmem_limit_bytes=vmem_limit,
                                      disable_semaphore_checks=True)
    except TypeError:
        params = pltpu.CompilerParams(vmem_limit_bytes=vmem_limit)
    out = pl.pallas_call(
        _kernel,
        in_specs=[any_spec] * 10,
        out_specs=any_spec,
        out_shape=jax.ShapeDtypeStruct((M, 2 * D), BF16),
        scratch_shapes=[
            pltpu.VMEM((2, M, D), BF16),
            pltpu.VMEM((NSTEP - 1, B, S, DH), BF16),
            pltpu.VMEM((NSTEP - 1, B, S, DH), BF16),
            pltpu.VMEM((NSTEP, B, HG, S, DH), BF16),
            pltpu.VMEM((NSTEP, B, HG, S, DH), BF16),
            pltpu.VMEM((D, 3 * W), BF16),
            pltpu.VMEM((NSTEP - 1, D, W), BF16),
            pltpu.VMEM((NSTEP - 2, D, W), BF16),
            pltpu.VMEM((NSTEP, W, D), BF16), pltpu.VMEM((NSTEP, W, D), BF16),
            pltpu.VMEM((M, 3 * W), F32),
            pltpu.VMEM((M, W), BF16), pltpu.VMEM((M, W), BF16),
            pltpu.VMEM((M, 2 * D), F32),
            pltpu.VMEM((M, D), BF16), pltpu.VMEM((M, D), BF16),
            pltpu.SemaphoreType.DMA((NSEM,)),
        ],
        compiler_params=params,
    )(A_x.reshape(M, D), A_k_cache, A_v_cache, A_wq, A_wo,
      B_x.reshape(M, D), B_k_cache, B_v_cache, B_wq, B_wo)
    return out.reshape(B, S, 2 * D)
```
